```python
import os as _os
_os.environ.setdefault("JAX_PLATFORMS", "cpu")
import jax
import jax.numpy as jnp

def _softmax(x, axis=-1):
    return jax.nn.softmax(x, axis=axis)
def _gelu(x):
    return jax.nn.gelu(x, approximate=True)
def _silu(x):
    return jax.nn.silu(x)
def _sigmoid(x):
    return jax.nn.sigmoid(x)
def _layernorm(x, axis=-1, eps=1e-5):
    m = jnp.mean(x, axis=axis, keepdims=True)
    v = jnp.var(x, axis=axis, keepdims=True)
    return (x - m) / jnp.sqrt(v + eps)
def _scatter_add(tgt, idx, src, axis=0):
    return tgt.at[idx].add(src)
def _segment_sum(src, seg, n):
    return jax.ops.segment_sum(src, seg, n)
class _Rng:
    def __init__(self, key):
        self._k = key
    def _next(self):
        self._k, sub = jax.random.split(self._k)
        return sub
    def normal(self, shape):
        return jax.random.normal(self._next(), shape, dtype=jnp.bfloat16)
    def randint(self, lo, hi, shape):
        return jax.random.randint(self._next(), shape, lo, hi, dtype=jnp.int32)
    def uniform(self, shape, lo=0.0, hi=1.0):
        return jax.random.uniform(self._next(), shape, jnp.bfloat16, lo, hi)
    def permutation(self, n):
        return jax.random.permutation(self._next(), n)


kernel_name = 'standalone__gqa_block_cached__near_ridge'

def setup_inputs():
    _rng = _Rng(jax.random.key(int.from_bytes(__import__("os").urandom(4), "little")))
    _w = (lambda a: (lambda t: t.astype(jnp.bfloat16) if jnp.issubdtype(t.dtype, jnp.floating) else t)(jnp.asarray(a)))
    B, Sq, D = 8, 80, 512
    Hq, Hkv, Sk, Dh = 32, 8, 2048, 128
    assert Hq % Hkv == 0, (Hq, Hkv)
    return {
        "x": _w((lambda *s: _rng.normal(s) * 0.8)(B, Sq, D)),
        "k_cache": _w((lambda *s: _rng.normal(s) * 0.8)(B, Hkv, Sk, Dh)),
        "v_cache": _w((lambda *s: _rng.normal(s) * 0.05)(B, Hkv, Sk, Dh)),
        "wq": _w((lambda *s: _rng.normal(s) * 0.8)(D, Hq * Dh) * (D ** -0.5)),
        "wo": _w((lambda *s: _rng.normal(s) * 0.05)(Hq * Dh, D) * ((Hq * Dh) ** -0.5)),
    }

def reference(x, k_cache, v_cache, wq, wo):
    B, Sq, D = x.shape
    Hq, Dh = 32, 128
    Hkv = k_cache.shape[1]
    rep = Hq // Hkv
    q = (lambda x, *d: x.transpose(*d))((x @ wq).reshape(B, Sq, Hq, Dh), 0, 2, 1, 3)
    k = jnp.repeat(k_cache, rep, axis=1)
    v = jnp.repeat(v_cache, rep, axis=1)
    scores = jnp.einsum("bhqd,bhkd->bhqk", q, k) * (Dh ** -0.5)
    p = _softmax(scores, axis=-1)
    o = jnp.einsum("bhqk,bhkd->bhqd", p, v)
    return (lambda x, *d: x.transpose(*d))(o, 0, 2, 1, 3).reshape(B, Sq, Hq * Dh) @ wo
```

```python
import functools
import jax
import jax.numpy as jnp
from jax import lax
import jax.experimental.pallas as pl
import jax.experimental.pallas.tpu as pltpu

B, SQ, D = 8, 80, 512
HQ, HKV, SK, DH = 32, 8, 2048, 128
REP = HQ // HKV
M = REP * SQ
NU = B * HKV
R = B * SQ
LOG2E = 1.4426950408889634
SCALE = (DH ** -0.5) * LOG2E
NT = (((1,), (1,)), ((), ()))
F32 = jnp.float32
BF16 = jnp.bfloat16
U32 = jnp.uint32


def make(U=8, CK=512, NG=3, CUT=3, lp=True, flags=None, nobc=True, WQ=(4, 8, 20), WOI=2,
         p1='col', p3='col', P3K=512, P3R=640, opaque=False, split0=True):
    assert NU % U == 0 and U % 2 == 0
    NCH = SK // CK
    NIT = NU // U
    flags = dict(flags or {})
    if lp:
        flags['XLA_TPU_FORCE_LP_LLO_SCHEDULER'] = True
    NSLOT = NG * U
    PER = 2 * NCH

    def kernel(x_hbm, k_hbm, v_hbm, wq_hbm, wo_hbm, o_hbm,
               x_s, kbuf, vbuf, wq_s, wo_s, q_s, a_s, o_s, s0, s1, m0, m1, acc_s, l_s, mr_s, oacc_s,
               ksem, vsem, wqsem, msem, osem, zsem):
        sbufs = (s0, s1)
        mbufs = (m0, m1)

        def ld(ref, idx, r0, n, cols=slice(None)):
            h0 = r0 // 2
            w = ref.bitcast(U32)[(*idx, pl.ds(h0, n // 2), cols)]
            return pltpu.bitcast(w, BF16)

        def k_cp(g, n=U):
            s = g % NG
            return pltpu.make_async_copy(k_hbm.at[pl.ds(g * U + 1, n)], kbuf.at[pl.ds(s * U + 1, n)], ksem.at[s])

        def v_cp(g):
            s = g % NG
            return pltpu.make_async_copy(v_hbm.at[pl.ds(g * U, U)], vbuf.at[pl.ds(s * U, U)], vsem.at[s])

        H0 = U // 2
        k0a = pltpu.make_async_copy(k_hbm.at[pl.ds(0, H0 + 1)], kbuf.at[pl.ds(0, H0 + 1)], msem.at[0])
        v0a = pltpu.make_async_copy(v_hbm.at[pl.ds(0, H0)], vbuf.at[pl.ds(0, H0)], msem.at[3])
        k0b = pltpu.make_async_copy(k_hbm.at[pl.ds(H0 + 1, U - H0)], kbuf.at[pl.ds(H0 + 1, U - H0)], ksem.at[0])
        v0b = pltpu.make_async_copy(v_hbm.at[pl.ds(H0, U - H0)], vbuf.at[pl.ds(H0, U - H0)], vsem.at[0])
        def slab_start(hbm, vmem, c0, c1, sem, priority=0):
            for c in range(c0, c1):
                pltpu.make_async_copy(hbm.at[:, pl.ds(c * 128, 128)], vmem.at[c], sem).start(priority=priority)

        def slab_wait(vmem, c0, c1, sem):
            pltpu.make_async_copy(vmem.at[pl.ds(c0, c1 - c0)], vmem.at[pl.ds(c0, c1 - c0)], sem).wait()

        wq_offs = [sum(WQ[:i]) for i in range(len(WQ))]

        def wq_start(i, priority):
            slab_start(wq_hbm, wq_s, wq_offs[i], wq_offs[i] + WQ[i], wqsem.at[i], priority)

        def wq_wait(i):
            slab_wait(wq_s, wq_offs[i], wq_offs[i] + WQ[i], wqsem.at[i])

        slab_start(x_hbm, x_s, 0, 4, msem.at[1])
        wq_start(0, 0)
        wq_start(1, 1)
        zero = pl.semaphore_read(zsem.at[0]) if opaque else 0

        with jax.named_scope("wait_x"):
            slab_wait(x_s, 0, 4, msem.at[1])
            wq_wait(0)
        for i in range(len(WQ)):
          with jax.named_scope(f"p1_{i}"):
            if i > 0:
                wq_wait(i)
            if i + 2 < len(WQ):
                wq_start(i + 2, 1)
            if i == len(WQ) - 1:
                k0a.start()
                v0a.start()
                k0b.start(priority=1)
                v0b.start(priority=1)
            if p1 == 'col':
                for hq in range(wq_offs[i], wq_offs[i] + WQ[i]):
                    h, g = divmod(hq, REP)
                    r0 = pl.multiple_of(zero * hq, 8) if opaque else 0
                    xv = jnp.concatenate([pltpu.bitcast(x_s.bitcast(U32)[c, pl.ds(r0, R // 2), :], BF16) for c in range(4)], axis=1)
                    q = jnp.dot(xv, ld(wq_s, (hq,), 0, D), preferred_element_type=F32) * SCALE
                    q = pltpu.bitcast(q.astype(BF16), U32)
                    for b in range(B):
                        q_s[b * HKV + h, g * SQ // 2:(g + 1) * SQ // 2, :] = q[b * SQ // 2:(b + 1) * SQ // 2]
            else:
                for h in range(wq_offs[i] // REP, (wq_offs[i] + WQ[i]) // REP):
                    r0 = pl.multiple_of(zero * h, 8) if opaque else 0
                    xv = jnp.concatenate([pltpu.bitcast(x_s.bitcast(U32)[c, pl.ds(r0, R // 2), :], BF16) for c in range(4)], axis=1)
                    w = jnp.concatenate([ld(wq_s, (h * REP + g,), 0, D) for g in range(REP)], axis=1)
                    q = jnp.dot(xv, w, preferred_element_type=F32) * SCALE
                    q = pltpu.bitcast(q.astype(BF16), U32)
                    for b in range(B):
                        for g in range(REP):
                            q_s[b * HKV + h, g * SQ // 2:(g + 1) * SQ // 2, :] = q[b * SQ // 2:(b + 1) * SQ // 2, g * DH:(g + 1) * DH]

        def qk_chunk(u, slot, par, j):
            q = pltpu.bitcast(q_s[u], BF16)
            k = ld(kbuf, (slot,), j * CK, CK)
            s = lax.dot_general(q, k, NT, preferred_element_type=F32)
            sbufs[par][:, j * CK:(j + 1) * CK] = s
            mrun = mr_s[...] if j > 0 else None
            for c in range(CK // 128):
                t = s[:, c * 128:(c + 1) * 128]
                mrun = t if mrun is None else jnp.maximum(mrun, t)
            if j < NCH - 1:
                mr_s[...] = mrun
            else:
                m = jnp.max(mrun, axis=1, keepdims=True)
                mbufs[par][...] = jnp.broadcast_to(m, (M, 128))

        def pv_chunk(u, slot, par, j):
            m = mbufs[par][...]
            ps = []
            lrun = l_s[...] if j > 0 else None
            for c in range(CK // 128):
                s = sbufs[par][:, j * CK + c * 128:j * CK + (c + 1) * 128]
                p = jnp.exp2(s - m)
                lrun = p if lrun is None else lrun + p
                ps.append(p)
            if j < NCH - 1:
                l_s[...] = lrun
            p = jnp.concatenate(ps, axis=1).astype(BF16)
            v = ld(vbuf, (slot,), j * CK, CK)
            o = jnp.dot(p, v, preferred_element_type=F32)
            if j > 0:
                o = o + acc_s[...]
            if j < NCH - 1:
                acc_s[...] = o
            else:
                l = jnp.sum(lrun, axis=1, keepdims=True)
                r = pltpu.reciprocal(l, approx=True)
                r = r * (2.0 - l * r)
                o = o * r
                o = jnp.concatenate([o[g * SQ:(g + 1) * SQ, :] for g in range(REP)], axis=1)
                b = u // HKV
                h = u % HKV
                r0 = b * (SQ // 2) if isinstance(b, int) else pl.multiple_of(b * (SQ // 2), 8)
                a_s[h, pl.ds(r0, SQ // 2), :] = pltpu.bitcast(o.astype(BF16), U32)

        def run_ops(base, lo, hi, has_q=lambda d: True, has_v=lambda d: True):
            sb = base % NSLOT
            for p in range(lo, hi):
                d, r = divmod(p, PER)
                j = r // 2
                slot = (sb + NSLOT - 1) % NSLOT if d == 0 else sb + d - 1
                if r % 2 == 0:
                    if has_q(d):
                        u = base + d
                        qk_chunk(u, 0 if (isinstance(u, int) and u == 0) else slot + 1, d % 2, j)
                elif has_v(d):
                    pv_chunk(base + d - 1, slot, (d + 1) % 2, j)

        def start_group(g):
            @pl.when(g < NIT - 1)
            def _():
                k_cp(g).start()

            @pl.when(g == NIT - 1)
            def _():
                k_cp(g, U - 1).start()

            @pl.when(g < NIT)
            def _():
                v_cp(g).start()

        with jax.named_scope("wait_g0a"):
            k0a.wait()
            v0a.wait()
        with jax.named_scope("first_a"):
            for g in range(1, NG - 1):
                k_cp(g).start(priority=1)
                v_cp(g).start(priority=1)
            run_ops(0, 0, CUT + H0 * PER, has_v=lambda d: d > 0)
        with jax.named_scope("wait_g0b"):
            k0b.wait()
            v0b.wait()
        with jax.named_scope("first_b"):
            run_ops(0, CUT + H0 * PER, CUT + U * PER)

        def body(i, carry):
            with jax.named_scope("loopwait"):
                k_cp(i).wait()
                v_cp(i).wait()
            start_group(i + NG - 2)

            @pl.when(i == WOI)
            def _():
                slab_start(wo_hbm, wo_s, 0, 4, msem.at[2], 1)

            with jax.named_scope("loopbody"):
                run_ops(i * U, CUT, CUT + U * PER)
            return carry

        lax.fori_loop(1, NIT - 1, body, 0)

        i = NIT - 1
        with jax.named_scope("lastwait"):
            k_cp(i, U - 1).wait()
            v_cp(i).wait()
            slab_wait(wo_s, 0, 4, msem.at[2])
        with jax.named_scope("last"):
            run_ops(i * U, CUT, (U + 1) * PER, has_q=lambda d: d < U)

        ocps = []
        with jax.named_scope("p3"):
            if p3 == 'col':
                for n in range(D // 128):
                    cols = pl.ds(n * 128, 128)
                    NK = HQ * DH // P3K
                    for kc in range(NK):
                        hs = range(kc * P3K // 512, (kc + 1) * P3K // 512)
                        a = jnp.concatenate([pltpu.bitcast(a_s[h], BF16) for h in hs], axis=1)
                        d = jnp.dot(a, ld(wo_s, (n,), kc * P3K, P3K), preferred_element_type=F32)
                        if kc > 0:
                            d = d + oacc_s[...]
                        if kc < NK - 1:
                            oacc_s[...] = d
                    o_s.bitcast(U32)[n] = pltpu.bitcast(d.astype(BF16), U32)
                    cp = pltpu.make_async_copy(o_s.at[n], o_hbm.at[:, cols], osem.at[n])
                    cp.start()
                    ocps.append(cp)
        with jax.named_scope("owait"):
            for cp in ocps:
                cp.wait()

    def fn(x, k_cache, v_cache, wq, wo):
        out = pl.pallas_call(
            kernel,
            out_shape=jax.ShapeDtypeStruct((R, D), BF16),
            in_specs=[pl.BlockSpec(memory_space=pl.ANY)] * 5,
            out_specs=pl.BlockSpec(memory_space=pl.ANY),
            scratch_shapes=[
                pltpu.VMEM((D // 128, R, 128), BF16),
                pltpu.VMEM((NSLOT + 1, SK, DH), BF16),
                pltpu.VMEM((NSLOT, SK, DH), BF16),
                pltpu.VMEM((HQ, D, DH), BF16),
                pltpu.VMEM((D // 128, HQ * DH, 128), BF16),
                pltpu.VMEM((NU, M // 2, DH), U32),
                pltpu.VMEM((HKV, R // 2, REP * DH), U32),
                pltpu.VMEM((D // 128, R, 128), BF16),
                pltpu.VMEM((M, SK), F32),
                pltpu.VMEM((M, SK), F32),
                pltpu.VMEM((M, 128), F32),
                pltpu.VMEM((M, 128), F32),
                pltpu.VMEM((M, 128), F32),
                pltpu.VMEM((M, 128), F32),
                pltpu.VMEM((M, 128), F32),
                pltpu.VMEM((R, 128), F32),
                pltpu.SemaphoreType.DMA((NG,)),
                pltpu.SemaphoreType.DMA((NG,)),
                pltpu.SemaphoreType.DMA((len(WQ),)),
                pltpu.SemaphoreType.DMA((4,)),
                pltpu.SemaphoreType.DMA((8,)),
                pltpu.SemaphoreType.REGULAR((1,)),
            ],
            compiler_params=pltpu.CompilerParams(vmem_limit_bytes=120 * 1024 * 1024, flags=flags,
                                                 disable_bounds_checks=nobc),
        )(x.reshape(R, D), k_cache.reshape(NU, SK, DH), v_cache.reshape(NU, SK, DH), wq, wo)
        return out.reshape(B, SQ, D)
    return fn


@jax.jit
def pallas_standalone__gqa_block_cached__near_ridge_kernel(x, k_cache, v_cache, wq, wo):
    return make(U=4)(x, k_cache, v_cache, wq, wo)
```

```python
import jax
import jax.numpy as jnp
from jax import lax
import jax.experimental.pallas as pl
import jax.experimental.pallas.tpu as pltpu

B, SQ, D = 8, 80, 512
HQ, HKV, SK, DH = 32, 8, 2048, 128
REP = HQ // HKV
M = REP * SQ
NU = B * HKV
R = B * SQ
CK = 512
NCH = SK // CK
PER = 2 * NCH
SCALE = DH ** -0.5 * 1.4426950408889634

HEAD, CUT, U, NLOOP = 3, 2, 6, 10
assert HEAD + NLOOP * U == NU - 1 and U % 2 == 0
OFF = HEAD + 1
NG = NLOOP + 1
T0 = 2 * REP
WQ = (10, 14)
GPOS = 12
OSPLIT = 4
NSLAB = D // 128

WQ0 = 0
K0 = WQ0 + HQ
V0 = K0 + NU * NCH
WO0 = V0 + NU * NCH
NSLOT = WO0 + HQ

F32, BF16, U32 = jnp.float32, jnp.bfloat16, jnp.uint32


def _kernel(x_hbm, k_hbm, v_hbm, wq_hbm, wo_hbm, o_hbm,
            xw_s, w_s, q_s, a_s, o_s, s0, s1, m0, m1, acc_s, l_s, mr_s, qacc_s, oacc_s,
            kvsem, xsem, wqsem, osem):
    s_bufs, m_bufs = (s0, s1), (m0, m1)

    def load(ref, i, r0, n):
        return pltpu.bitcast(ref.at[i, pl.ds(r0, n)].bitcast(U32)[...], BF16)

    def pack(v):
        return pltpu.bitcast(v.astype(BF16), U32)

    def weights(slot):
        return load(w_s, slot, 0, CK)

    def start(copies, priority=1):
        for c in copies:
            c.start(priority=priority)

    def wait(copies):
        for c in copies:
            c.wait()

    def kv_copy(src, base, u0, n, sem):
        return pltpu.make_async_copy(
            src.at[pl.ds(u0 * NCH, n * NCH)], w_s.at[pl.ds(base + u0 * NCH, n * NCH)], sem)

    def kv_group(g):
        if isinstance(g, int) and g == 0:
            return (kv_copy(k_hbm, K0, 0, OFF, kvsem.at[0]),
                    kv_copy(v_hbm, V0, 0, OFF - 1, kvsem.at[0]))
        d = OFF + (g - 1) * U
        return (kv_copy(k_hbm, K0, d, U, kvsem.at[g]),
                kv_copy(v_hbm, V0, d - 1, U, kvsem.at[g]))

    def tail_group():
        copies = [kv_copy(v_hbm, V0, NU - 1, 1, kvsem.at[NG])]
        for n in range(NSLAB):
            copies.append(pltpu.make_async_copy(
                wo_hbm.at[:, :, pl.ds(n * 128, 128)], w_s.at[pl.ds(WO0 + n * HKV, HKV)],
                kvsem.at[NG]))
        return copies

    def x_stage(i):
        copies = [pltpu.make_async_copy(
            x_hbm.at[:, pl.ds(i * 128, 128)], xw_s.at[i, pl.ds(0, R)], xsem.at[i])]
        for t in range(T0):
            copies.append(pltpu.make_async_copy(
                wq_hbm.at[pl.ds(i * 128, 128), pl.ds(t * DH, DH)],
                xw_s.at[t % REP, pl.ds(R + (t // REP) * D + i * 128, 128)], xsem.at[i]))
        return copies

    wq_first = [T0 + sum(WQ[:i]) for i in range(len(WQ))]
    for i in range(NSLAB):
        start(x_stage(i), priority=0)
    for i, (t0, n) in enumerate(zip(wq_first, WQ)):
        start([pltpu.make_async_copy(wq_hbm.at[:, pl.ds(t * DH, DH)], w_s.at[WQ0 + t], wqsem.at[i])
               for t in range(t0, t0 + n)])
    start(kv_group(0))

    def store_q(q, h, g):
        for b in range(B):
            q_s[b * HKV + h, g * SQ // 2:(g + 1) * SQ // 2, :] = q[b * SQ // 2:(b + 1) * SQ // 2]

    for i in range(NSLAB):
        wait(x_stage(i))
        x = load(xw_s, i, 0, R)
        for h in range(T0 // REP):
            w = jnp.concatenate(
                [load(xw_s, g, R + h * D + i * 128, 128) for g in range(REP)], axis=1)
            q = jnp.dot(x, w, preferred_element_type=F32)
            if i > 0:
                q = q + qacc_s[h]
            if i < NSLAB - 1:
                qacc_s[h] = q
            else:
                q = pack(q * SCALE)
                for g in range(REP):
                    store_q(q[:, g * DH:(g + 1) * DH], h, g)

    for i, (t0, n) in enumerate(zip(wq_first, WQ)):
        batch = w_s.at[pl.ds(WQ0 + t0, n)]
        pltpu.make_async_copy(batch, batch, wqsem.at[i]).wait()
        for t in range(t0, t0 + n):
            if t == GPOS:
                start(kv_group(1))
            x = jnp.concatenate([load(xw_s, c, 0, R) for c in range(NSLAB)], axis=1)
            q = jnp.dot(x, weights(WQ0 + t), preferred_element_type=F32)
            store_q(pack(q * SCALE), t // REP, t % REP)

    def qk_op(u, par, j):
        q = pltpu.bitcast(q_s[u], BF16)
        s = lax.dot_general(q, weights(K0 + u * NCH + j), (((1,), (1,)), ((), ())),
                            preferred_element_type=F32)
        s_bufs[par][:, j * CK:(j + 1) * CK] = s
        m = mr_s[...] if j > 0 else None
        for c in range(CK // 128):
            t = s[:, c * 128:(c + 1) * 128]
            m = t if m is None else jnp.maximum(m, t)
        if j < NCH - 1:
            mr_s[...] = m
        else:
            m_bufs[par][...] = jnp.broadcast_to(jnp.max(m, axis=1, keepdims=True), (M, 128))

    def pv_op(u, par, j):
        m = m_bufs[par][...]
        l = l_s[...] if j > 0 else None
        ps = []
        for c in range(CK // 128):
            p = jnp.exp2(s_bufs[par][:, j * CK + c * 128:j * CK + (c + 1) * 128] - m)
            l = p if l is None else l + p
            ps.append(p)
        if j < NCH - 1:
            l_s[...] = l
        p = jnp.concatenate(ps, axis=1).astype(BF16)
        o = jnp.dot(p, weights(V0 + u * NCH + j), preferred_element_type=F32)
        if j > 0:
            o = o + acc_s[...]
        if j < NCH - 1:
            acc_s[...] = o
        else:
            r = pltpu.reciprocal(jnp.sum(l, axis=1, keepdims=True), approx=False, full_range=False)
            l_s[...] = jnp.broadcast_to(r, (M, 128))
            o = o * r
            a_s[u] = pack(jnp.concatenate([o[g * SQ:(g + 1) * SQ] for g in range(REP)], axis=1))

    def enter_group(g):
        wait(kv_group(g))
        if not isinstance(g, int):
            @pl.when(g + 1 < NG)
            def _():
                start(kv_group(g + 1))

            @pl.when(g + 1 == NG)
            def _():
                start(tail_group())

    def run_ops(d0, lo, hi, it=0):
        for pos in range(lo, hi):
            d, r = d0 + pos // PER, pos % PER
            u = d + it * U
            first = isinstance(u, int) and u == 0
            last = isinstance(u, int) and u == NU
            if r == 0:
                if last:
                    wait(tail_group())
                elif first:
                    enter_group(0)
                elif d >= OFF and (d - OFF) % U == 0:
                    enter_group((d - OFF) // U + 1 + it)
            if r % 2 == 0:
                if not first:
                    pv_op(u - 1, (d + 1) % 2, r // 2)
            elif not last:
                qk_op(u, d % 2, r // 2)

    run_ops(0, 0, HEAD * PER + CUT)

    def body(it, carry):
        run_ops(HEAD, CUT, U * PER + CUT, it)
        return carry

    lax.fori_loop(0, NLOOP, body, 0)

    def out_op(n, h, b0=0, nb=B):
        rows = pl.ds(b0 * SQ, nb * SQ)
        a = jnp.concatenate(
            [pltpu.bitcast(a_s[b * HKV + h], BF16) for b in range(b0, b0 + nb)], axis=0)
        o = jnp.dot(a, weights(WO0 + n * HKV + h), preferred_element_type=F32)
        if h > 0:
            o = o + oacc_s[rows, :]
        if h < HKV - 1:
            oacc_s[rows, :] = o
        else:
            o_s.at[n, rows].bitcast(U32)[...] = pack(o)
            pltpu.make_async_copy(
                o_s.at[n, rows], o_hbm.at[rows, pl.ds(n * 128, 128)], osem.at[0]).start()

    todo = [(n, h) for n in range(NSLAB) for h in range(HKV)]
    run_ops(NU - 1, CUT, PER + 1)
    for pos in range(PER + 2, 2 * PER, 2):
        out_op(*todo.pop(0))
        run_ops(NU - 1, pos, pos + 1)
    for n, h in todo[:-1]:
        out_op(n, h)
    for i in range(OSPLIT):
        out_op(*todo[-1], i * (B // OSPLIT), B // OSPLIT)
    pltpu.make_async_copy(o_s, o_s, osem.at[0]).wait()


@jax.jit
def pallas_standalone__gqa_block_cached__near_ridge_kernel(
    x: jax.Array,
    k_cache: jax.Array,
    v_cache: jax.Array,
    wq: jax.Array,
    wo: jax.Array,
):
    out = pl.pallas_call(
        _kernel,
        out_shape=jax.ShapeDtypeStruct((R, D), BF16),
        in_specs=[pl.BlockSpec(memory_space=pl.ANY)] * 5,
        out_specs=pl.BlockSpec(memory_space=pl.ANY),
        scratch_shapes=[
            pltpu.VMEM((NSLAB, R + D * T0 // REP, 128), BF16),
            pltpu.VMEM((NSLOT, CK, DH), BF16),
            pltpu.VMEM((NU, M // 2, DH), U32),
            pltpu.VMEM((NU, SQ // 2, REP * DH), U32),
            pltpu.VMEM((NSLAB, R, 128), BF16),
            pltpu.VMEM((M, SK), F32),
            pltpu.VMEM((M, SK), F32),
            pltpu.VMEM((M, 128), F32),
            pltpu.VMEM((M, 128), F32),
            pltpu.VMEM((M, 128), F32),
            pltpu.VMEM((M, 128), F32),
            pltpu.VMEM((M, 128), F32),
            pltpu.VMEM((T0 // REP, R, REP * DH), F32),
            pltpu.VMEM((R, 128), F32),
            pltpu.SemaphoreType.DMA((NG + 1,)),
            pltpu.SemaphoreType.DMA((NSLAB,)),
            pltpu.SemaphoreType.DMA((len(WQ),)),
            pltpu.SemaphoreType.DMA((1,)),
        ],
        compiler_params=pltpu.CompilerParams(
            vmem_limit_bytes=120 * 1024 * 1024,
            disable_bounds_checks=True,
            flags={
                "XLA_TPU_FORCE_LP_LLO_SCHEDULER": True,
                "XLA_TPU_RESCHEDULE_DMA_DONES": True,
            },
        ),
    )(
        x.reshape(R, D),
        k_cache.reshape(NU * NCH, CK, DH),
        v_cache.reshape(NU * NCH, CK, DH),
        wq,
        wo.reshape(HKV, CK, D),
    )
    return out.reshape(B, SQ, D)
```

```python
import jax
import jax.numpy as jnp
from jax import lax
import jax.experimental.pallas as pl
import jax.experimental.pallas.tpu as pltpu

B, SQ, D = 8, 80, 512
HQ, HKV, SK, DH = 32, 8, 2048, 128
REP = HQ // HKV
M = REP * SQ
NU = B * HKV
R = B * SQ
CK = 512
NCH = SK // CK
PER = 2 * NCH
SCALE = DH ** -0.5 * 1.4426950408889634

HEAD, CUT, U, NLOOP = 3, 2, 6, 10
assert HEAD + NLOOP * U == NU - 1 and U % 2 == 0
OFF = HEAD + 1
NG = NLOOP + 1
T0 = 2 * REP
WQ = (9, 15)
GPOS = 12
OSPLIT = 4
NSLAB = D // 128

WQ0 = 0
K0 = WQ0 + HQ
V0 = K0 + NU * NCH
WO0 = V0 + NU * NCH
NSLOT = WO0 + HQ

F32, BF16 = jnp.float32, jnp.bfloat16


def _kernel(x_hbm, k_hbm, v_hbm, wq_hbm, wo_hbm, o_hbm,
            xw_s, w_s, q_s, a_s, o_s, s0, s1, m0, m1, acc_s, l_s, mr_s, qacc_s, oacc_s,
            kvsem, xsem, wqsem, osem):
    s_bufs, m_bufs = (s0, s1), (m0, m1)

    def start(copies, priority=1):
        for c in copies:
            c.start(priority=priority)

    def wait(copies):
        for c in copies:
            c.wait()

    def kv_copy(src, base, u0, n, sem):
        return pltpu.make_async_copy(
            src.at[pl.ds(u0 * NCH, n * NCH)], w_s.at[pl.ds(base + u0 * NCH, n * NCH)], sem)

    def kv_group(g):
        if isinstance(g, int) and g == 0:
            return (kv_copy(k_hbm, K0, 0, OFF, kvsem.at[0]),
                    kv_copy(v_hbm, V0, 0, OFF - 1, kvsem.at[0]))
        d = OFF + (g - 1) * U
        return (kv_copy(k_hbm, K0, d, U, kvsem.at[1]),
                kv_copy(v_hbm, V0, d - 1, U, kvsem.at[1]))

    def tail_group():
        copies = [kv_copy(v_hbm, V0, NU - 1, 1, kvsem.at[2])]
        for n in range(NSLAB):
            copies.append(pltpu.make_async_copy(
                wo_hbm.at[:, :, pl.ds(n * 128, 128)], w_s.at[pl.ds(WO0 + n * HKV, HKV)],
                kvsem.at[2]))
        return copies

    def x_stage(i):
        copies = [pltpu.make_async_copy(
            x_hbm.at[:, pl.ds(i * 128, 128)], xw_s.at[i, pl.ds(0, R)], xsem.at[i])]
        for t in range(T0):
            copies.append(pltpu.make_async_copy(
                wq_hbm.at[pl.ds(i * 128, 128), pl.ds(t * DH, DH)],
                xw_s.at[t % REP, pl.ds(R + (t // REP) * D + i * 128, 128)], xsem.at[i]))
        return copies

    wq_first = [T0 + sum(WQ[:i]) for i in range(len(WQ))]
    for i in range(NSLAB):
        start(x_stage(i), priority=0)
    for i, (t0, n) in enumerate(zip(wq_first, WQ)):
        start([pltpu.make_async_copy(wq_hbm.at[:, pl.ds(t * DH, DH)], w_s.at[WQ0 + t], wqsem.at[i])
               for t in range(t0, t0 + n)])
    start(kv_group(0))

    def store_q(q, h, g):
        for b in range(B):
            q_s[b * HKV + h, g * SQ:(g + 1) * SQ, :] = q[b * SQ:(b + 1) * SQ]

    for i in range(NSLAB):
        wait(x_stage(i))
        x = xw_s[i, 0:R, :]
        for h in range(T0 // REP):
            r0 = R + h * D + i * 128
            w = jnp.concatenate([xw_s[g, r0:r0 + 128, :] for g in range(REP)], axis=1)
            q = jnp.dot(x, w, preferred_element_type=F32)
            if i > 0:
                q = q + qacc_s[h]
            if i < NSLAB - 1:
                qacc_s[h] = q
            else:
                q = (q * SCALE).astype(BF16)
                for g in range(REP):
                    store_q(q[:, g * DH:(g + 1) * DH], h, g)

    for i, (t0, n) in enumerate(zip(wq_first, WQ)):
        batch = w_s.at[pl.ds(WQ0 + t0, n)]
        pltpu.make_async_copy(batch, batch, wqsem.at[i]).wait()
        for t in range(t0, t0 + n):
            if t == GPOS:
                start(kv_group(1))
            x = jnp.concatenate([xw_s[c, 0:R, :] for c in range(NSLAB)], axis=1)
            q = jnp.dot(x, w_s[WQ0 + t], preferred_element_type=F32)
            store_q((q * SCALE).astype(BF16), t // REP, t % REP)

    def qk_op(u, par, j):
        s = lax.dot_general(q_s[u], w_s[K0 + u * NCH + j], (((1,), (1,)), ((), ())),
                            preferred_element_type=F32)
        s_bufs[par][:, j * CK:(j + 1) * CK] = s
        m = mr_s[...] if j > 0 else None
        for c in range(CK // 128):
            t = s[:, c * 128:(c + 1) * 128]
            m = t if m is None else jnp.maximum(m, t)
        if j < NCH - 1:
            mr_s[...] = m
        else:
            m_bufs[par][...] = jnp.broadcast_to(jnp.max(m, axis=1, keepdims=True), (M, 128))

    def pv_op(u, par, j):
        m = m_bufs[par][...]
        l = l_s[...] if j > 0 else None
        ps = []
        for c in range(CK // 128):
            p = jnp.exp2(s_bufs[par][:, j * CK + c * 128:j * CK + (c + 1) * 128] - m)
            l = p if l is None else l + p
            ps.append(p)
        if j < NCH - 1:
            l_s[...] = l
        p = jnp.concatenate(ps, axis=1).astype(BF16)
        o = jnp.dot(p, w_s[V0 + u * NCH + j], preferred_element_type=F32)
        if j > 0:
            o = o + acc_s[...]
        if j < NCH - 1:
            acc_s[...] = o
        else:
            r = pltpu.reciprocal(jnp.sum(l, axis=1, keepdims=True), approx=False, full_range=False)
            l_s[...] = jnp.broadcast_to(r, (M, 128))
            o = o * r
            o = jnp.concatenate([o[g * SQ:(g + 1) * SQ] for g in range(REP)], axis=1)
            a_s[u] = o.astype(BF16)

    def run_ops(d0, lo, hi, it=0):
        for pos in range(lo, hi):
            d, r = d0 + pos // PER, pos % PER
            u = d + it * U
            in_loop = not isinstance(u, int)
            if in_loop and d == OFF and r == 0:
                wait(kv_group(it + 1))
            if in_loop and d == OFF and r == 2:
                @pl.when(it + 2 < NG)
                def _():
                    start(kv_group(it + 2), priority=0)
            if r % 2 == 0:
                if in_loop or u > 0:
                    pv_op(u - 1, (d + 1) % 2, r // 2)
            elif in_loop or u < NU:
                qk_op(u, d % 2, r // 2)

    wait(kv_group(0))
    start(tail_group())
    run_ops(0, 0, HEAD * PER + CUT)

    def body(it, carry):
        run_ops(HEAD, CUT, U * PER + CUT, it)
        return carry

    lax.fori_loop(0, NLOOP, body, 0)

    def out_op(n, h, b0=0, nb=B):
        rows = pl.ds(b0 * SQ, nb * SQ)
        a = jnp.concatenate([a_s[b * HKV + h] for b in range(b0, b0 + nb)], axis=0)
        o = jnp.dot(a, w_s[WO0 + n * HKV + h], preferred_element_type=F32)
        if h > 0:
            o = o + oacc_s[rows, :]
        if h < HKV - 1:
            oacc_s[rows, :] = o
        else:
            o_s[n, rows, :] = o.astype(BF16)
            pltpu.make_async_copy(
                o_s.at[n, rows], o_hbm.at[rows, pl.ds(n * 128, 128)], osem.at[0]).start()

    todo = [(n, h) for n in range(NSLAB) for h in range(HKV)]
    run_ops(NU - 1, CUT, PER)
    wait(tail_group())
    run_ops(NU - 1, PER, PER + 1)
    for pos in range(PER + 2, 2 * PER, 2):
        out_op(*todo.pop(0))
        run_ops(NU - 1, pos, pos + 1)
    for n, h in todo[:-1]:
        out_op(n, h)
    for i in range(OSPLIT):
        out_op(*todo[-1], i * (B // OSPLIT), B // OSPLIT)
    pltpu.make_async_copy(o_s, o_s, osem.at[0]).wait()


@jax.jit
def pallas_standalone__gqa_block_cached__near_ridge_kernel(
    x: jax.Array,
    k_cache: jax.Array,
    v_cache: jax.Array,
    wq: jax.Array,
    wo: jax.Array,
):
    out = pl.pallas_call(
        _kernel,
        out_shape=jax.ShapeDtypeStruct((R, D), BF16),
        in_specs=[pl.BlockSpec(memory_space=pl.ANY)] * 5,
        out_specs=pl.BlockSpec(memory_space=pl.ANY),
        scratch_shapes=[
            pltpu.VMEM((NSLAB, R + D * T0 // REP, 128), BF16),
            pltpu.VMEM((NSLOT, CK, DH), BF16),
            pltpu.VMEM((NU, M, DH), BF16),
            pltpu.VMEM((NU, SQ, REP * DH), BF16),
            pltpu.VMEM((NSLAB, R, 128), BF16),
            pltpu.VMEM((M, SK), F32),
            pltpu.VMEM((M, SK), F32),
            pltpu.VMEM((M, 128), F32),
            pltpu.VMEM((M, 128), F32),
            pltpu.VMEM((M, 128), F32),
            pltpu.VMEM((M, 128), F32),
            pltpu.VMEM((M, 128), F32),
            pltpu.VMEM((T0 // REP, R, REP * DH), F32),
            pltpu.VMEM((R, 128), F32),
            pltpu.SemaphoreType.DMA((3,)),
            pltpu.SemaphoreType.DMA((NSLAB,)),
            pltpu.SemaphoreType.DMA((len(WQ),)),
            pltpu.SemaphoreType.DMA((1,)),
        ],
        compiler_params=pltpu.CompilerParams(
            vmem_limit_bytes=120 * 1024 * 1024,
            flags={
                "XLA_TPU_FORCE_LP_LLO_SCHEDULER": True,
                "XLA_TPU_RESCHEDULE_DMA_DONES": True,
            },
        ),
    )(
        x.reshape(R, D),
        k_cache.reshape(NU * NCH, CK, DH),
        v_cache.reshape(NU * NCH, CK, DH),
        wq,
        wo.reshape(HKV, CK, D),
    )
    return out.reshape(B, SQ, D)
```

```python
import jax
import jax.numpy as jnp
from jax import lax
import jax.experimental.pallas as pl
import jax.experimental.pallas.tpu as pltpu

B, SQ, D = 8, 80, 512
HQ, HKV, SK, DH = 32, 8, 2048, 128
REP = HQ // HKV
M = REP * SQ
NU = B * HKV
R = B * SQ
CK = 512
NCH = SK // CK
PER = 2 * NCH
SCALE = DH ** -0.5 * 1.4426950408889634

HEAD, CUT, U, NLOOP = 3, 2, 6, 10
assert HEAD + NLOOP * U == NU - 1 and U % 2 == 0
OFF = HEAD + 1
NG = NLOOP + 1
T0 = 2 * REP
WQ = (9, 15)
GPOS = 12
OSPLIT = 4
NSLAB = D // 128

WQ0 = 0
K0 = WQ0 + HQ
V0 = K0 + NU * NCH
WO0 = V0 + NU * NCH
NSLOT = WO0 + HQ

F32, BF16 = jnp.float32, jnp.bfloat16


def _kernel(x_hbm, k_hbm, v_hbm, wq_hbm, wo_hbm, o_hbm,
            xw_s, w_s, q_s, a_s, o_s, s0, s1, m0, m1, acc_s, l_s, mr_s, qacc_s, oacc_s,
            kvsem, xsem, wqsem, osem):
    s_bufs, m_bufs = (s0, s1), (m0, m1)

    def start(copies, priority=1):
        for c in copies:
            c.start(priority=priority)

    def wait(copies):
        for c in copies:
            c.wait()

    def kv_copy(src, base, u0, n, sem):
        return pltpu.make_async_copy(
            src.at[pl.ds(u0 * NCH, n * NCH)], w_s.at[pl.ds(base + u0 * NCH, n * NCH)], sem)

    def kv_group(g):
        if isinstance(g, int) and g == 0:
            return (kv_copy(k_hbm, K0, 0, OFF, kvsem.at[0]),
                    kv_copy(v_hbm, V0, 0, OFF - 1, kvsem.at[0]))
        d = OFF + (g - 1) * U
        return (kv_copy(k_hbm, K0, d, U, kvsem.at[1]),
                kv_copy(v_hbm, V0, d - 1, U, kvsem.at[1]))

    def tail_group():
        copies = [kv_copy(v_hbm, V0, NU - 1, 1, kvsem.at[2])]
        for n in range(NSLAB):
            copies.append(pltpu.make_async_copy(
                wo_hbm.at[:, :, pl.ds(n * 128, 128)], w_s.at[pl.ds(WO0 + n * HKV, HKV)],
                kvsem.at[2]))
        return copies

    def x_stage(i):
        copies = [pltpu.make_async_copy(
            x_hbm.at[:, pl.ds(i * 128, 128)], xw_s.at[i, pl.ds(0, R)], xsem.at[i])]
        for t in range(T0):
            copies.append(pltpu.make_async_copy(
                wq_hbm.at[pl.ds(i * 128, 128), pl.ds(t * DH, DH)],
                xw_s.at[t % REP, pl.ds(R + (t // REP) * D + i * 128, 128)], xsem.at[i]))
        return copies

    wq_first = [T0 + sum(WQ[:i]) for i in range(len(WQ))]
    for i in range(NSLAB):
        start(x_stage(i), priority=0)
    for i, (t0, n) in enumerate(zip(wq_first, WQ)):
        start([pltpu.make_async_copy(wq_hbm.at[:, pl.ds(t * DH, DH)], w_s.at[WQ0 + t], wqsem.at[i])
               for t in range(t0, t0 + n)])
    start(kv_group(0))

    def store_q(q, h, g):
        for b in range(B):
            q_s[b * HKV + h, g * SQ:(g + 1) * SQ, :] = q[b * SQ:(b + 1) * SQ]

    for i in range(NSLAB):
        wait(x_stage(i))
        x = xw_s[i, 0:R, :]
        for h in range(T0 // REP):
            r0 = R + h * D + i * 128
            w = jnp.concatenate([xw_s[g, r0:r0 + 128, :] for g in range(REP)], axis=1)
            q = jnp.dot(x, w, preferred_element_type=F32)
            if i > 0:
                q = q + qacc_s[h]
            if i < NSLAB - 1:
                qacc_s[h] = q
            else:
                q = (q * SCALE).astype(BF16)
                for g in range(REP):
                    store_q(q[:, g * DH:(g + 1) * DH], h, g)

    for i, (t0, n) in enumerate(zip(wq_first, WQ)):
        batch = w_s.at[pl.ds(WQ0 + t0, n)]
        pltpu.make_async_copy(batch, batch, wqsem.at[i]).wait()
        for t in range(t0, t0 + n):
            if t == GPOS:
                start(kv_group(1))
            x = jnp.concatenate([xw_s[c, 0:R, :] for c in range(NSLAB)], axis=1)
            q = jnp.dot(x, w_s[WQ0 + t], preferred_element_type=F32)
            store_q((q * SCALE).astype(BF16), t // REP, t % REP)

    def qk_op(u, par, j):
        s = lax.dot_general(q_s[u], w_s[K0 + u * NCH + j], (((1,), (1,)), ((), ())),
                            preferred_element_type=F32)
        s_bufs[par][:, j * CK:(j + 1) * CK] = s
        m = mr_s[...] if j > 0 else None
        for c in range(CK // 128):
            t = s[:, c * 128:(c + 1) * 128]
            m = t if m is None else jnp.maximum(m, t)
        if j < NCH - 1:
            mr_s[...] = m
        else:
            m_bufs[par][...] = jnp.broadcast_to(jnp.max(m, axis=1, keepdims=True), (M, 128))

    def pv_op(u, par, j):
        m = m_bufs[par][...]
        l = l_s[...] if j > 0 else None
        ps = []
        for c in range(CK // 128):
            p = jnp.exp2(s_bufs[par][:, j * CK + c * 128:j * CK + (c + 1) * 128] - m)
            l = p if l is None else l + p
            ps.append(p)
        if j < NCH - 1:
            l_s[...] = l
        p = jnp.concatenate(ps, axis=1).astype(BF16)
        o = jnp.dot(p, w_s[V0 + u * NCH + j], preferred_element_type=F32)
        if j > 0:
            o = o + acc_s[...]
        if j < NCH - 1:
            acc_s[...] = o
        else:
            r = pltpu.reciprocal(jnp.sum(l, axis=1, keepdims=True), approx=False, full_range=False)
            l_s[...] = jnp.broadcast_to(r, (M, 128))
            o = o * r
            o = jnp.concatenate([o[g * SQ:(g + 1) * SQ] for g in range(REP)], axis=1)
            a_s[u] = o.astype(BF16)

    def run_ops(d0, lo, hi, it=0):
        for pos in range(lo, hi):
            d, r = d0 + pos // PER, pos % PER
            u = d + it * U
            in_loop = not isinstance(u, int)
            if in_loop and d == OFF and r == 0:
                wait(kv_group(it + 1))
            if in_loop and d == OFF and r == 2:
                @pl.when(it + 2 < NG)
                def _():
                    start(kv_group(it + 2), priority=0)
            if r % 2 == 0:
                if in_loop or u > 0:
                    pv_op(u - 1, (d + 1) % 2, r // 2)
            elif in_loop or u < NU:
                qk_op(u, d % 2, r // 2)

    wait(kv_group(0))
    start(tail_group())
    run_ops(0, 0, HEAD * PER + CUT)

    def body(it, carry):
        run_ops(HEAD, CUT, U * PER + CUT, it)
        return carry

    lax.fori_loop(0, NLOOP, body, 0)

    out_copies = []

    def out_op(n, h, b0=0, nb=B):
        rows = pl.ds(b0 * SQ, nb * SQ)
        a = jnp.concatenate([a_s[b * HKV + h] for b in range(b0, b0 + nb)], axis=0)
        o = jnp.dot(a, w_s[WO0 + n * HKV + h], preferred_element_type=F32)
        if h > 0:
            o = o + oacc_s[rows, :]
        if h < HKV - 1:
            oacc_s[rows, :] = o
        else:
            o_s[n, rows, :] = o.astype(BF16)
            out_copies.append(pltpu.make_async_copy(
                o_s.at[n, rows], o_hbm.at[rows, pl.ds(n * 128, 128)], osem.at[0]))
            out_copies[-1].start()

    todo = [(n, h) for n in range(NSLAB) for h in range(HKV)]
    run_ops(NU - 1, CUT, PER)
    wait(tail_group())
    run_ops(NU - 1, PER, PER + 1)
    for pos in range(PER + 2, 2 * PER, 2):
        out_op(*todo.pop(0))
        run_ops(NU - 1, pos, pos + 1)
    for n, h in todo[:-1]:
        out_op(n, h)
    for i in range(OSPLIT):
        out_op(*todo[-1], i * (B // OSPLIT), B // OSPLIT)
    wait(out_copies)


@jax.jit
def pallas_standalone__gqa_block_cached__near_ridge_kernel(
    x: jax.Array,
    k_cache: jax.Array,
    v_cache: jax.Array,
    wq: jax.Array,
    wo: jax.Array,
):
    out = pl.pallas_call(
        _kernel,
        out_shape=jax.ShapeDtypeStruct((R, D), BF16),
        in_specs=[pl.BlockSpec(memory_space=pl.ANY)] * 5,
        out_specs=pl.BlockSpec(memory_space=pl.ANY),
        scratch_shapes=[
            pltpu.VMEM((NSLAB, R + D * T0 // REP, 128), BF16),
            pltpu.VMEM((NSLOT, CK, DH), BF16),
            pltpu.VMEM((NU, M, DH), BF16),
            pltpu.VMEM((NU, SQ, REP * DH), BF16),
            pltpu.VMEM((NSLAB, R, 128), BF16),
            pltpu.VMEM((M, SK), F32),
            pltpu.VMEM((M, SK), F32),
            pltpu.VMEM((M, 128), F32),
            pltpu.VMEM((M, 128), F32),
            pltpu.VMEM((M, 128), F32),
            pltpu.VMEM((M, 128), F32),
            pltpu.VMEM((M, 128), F32),
            pltpu.VMEM((T0 // REP, R, REP * DH), F32),
            pltpu.VMEM((R, 128), F32),
            pltpu.SemaphoreType.DMA((3,)),
            pltpu.SemaphoreType.DMA((NSLAB,)),
            pltpu.SemaphoreType.DMA((len(WQ),)),
            pltpu.SemaphoreType.DMA((1,)),
        ],
        compiler_params=pltpu.CompilerParams(
            vmem_limit_bytes=120 * 1024 * 1024,
            flags={
                "XLA_TPU_FORCE_LP_LLO_SCHEDULER": True,
                "XLA_TPU_RESCHEDULE_DMA_DONES": True,
            },
        ),
    )(
        x.reshape(R, D),
        k_cache.reshape(NU * NCH, CK, DH),
        v_cache.reshape(NU * NCH, CK, DH),
        wq,
        wo.reshape(HKV, CK, D),
    )
    return out.reshape(B, SQ, D)
```
